```python
import os as _os
_os.environ.setdefault("JAX_PLATFORMS", "cpu")
import jax
import jax.numpy as jnp

def _softmax(x, axis=-1):
    return jax.nn.softmax(x, axis=axis)
def _gelu(x):
    return jax.nn.gelu(x, approximate=True)
def _silu(x):
    return jax.nn.silu(x)
def _sigmoid(x):
    return jax.nn.sigmoid(x)
def _layernorm(x, axis=-1, eps=1e-5):
    m = jnp.mean(x, axis=axis, keepdims=True)
    v = jnp.var(x, axis=axis, keepdims=True)
    return (x - m) / jnp.sqrt(v + eps)
def _scatter_add(tgt, idx, src, axis=0):
    return tgt.at[idx].add(src)
def _segment_sum(src, seg, n):
    return jax.ops.segment_sum(src, seg, n)
class _Rng:
    def __init__(self, key):
        self._k = key
    def _next(self):
        self._k, sub = jax.random.split(self._k)
        return sub
    def normal(self, shape):
        return jax.random.normal(self._next(), shape, dtype=jnp.bfloat16)
    def randint(self, lo, hi, shape):
        return jax.random.randint(self._next(), shape, lo, hi, dtype=jnp.int32)
    def uniform(self, shape, lo=0.0, hi=1.0):
        return jax.random.uniform(self._next(), shape, jnp.bfloat16, lo, hi)
    def permutation(self, n):
        return jax.random.permutation(self._next(), n)


kernel_name = 'sequential_preLN__softmax_full_mha__swiglu_ffn__prompt'

def setup_inputs():
    _rng = _Rng(jax.random.key(int.from_bytes(__import__("os").urandom(4), "little")))
    _w = (lambda a: (lambda t: t.astype(jnp.bfloat16) if jnp.issubdtype(t.dtype, jnp.floating) else t)(jnp.asarray(a)))
    def _A_setup():
        B, S, D = 1, 2048, 512
        return {
            "x": _w((lambda *s: _rng.normal(s) * 0.05)(B, S, D)),
            "wqkv": _w((lambda *s: _rng.normal(s) * 0.05)(D, 3 * D)),
            "wo": _w((lambda *s: _rng.normal(s) * 0.05)(D, D)),
        }
    _A_in = _A_setup()

    def _B_setup():
        B, S, D, F = 1, 2048, 512, 1792
        return {
            "x": _w((lambda *s: _rng.normal(s) * 0.05)(B, S, D)),
            "w_gate": _w((lambda *s: _rng.normal(s) * 0.05)(D, F)),
            "w_up": _w((lambda *s: _rng.normal(s) * 0.05)(D, F)),
            "w_down": _w((lambda *s: _rng.normal(s) * 0.05)(F, D)),
        }
    _B_in = _B_setup()

    return {
        "A_x": _A_in["x"],
        "A_wqkv": _A_in["wqkv"],
        "A_wo": _A_in["wo"],
        "B_x": _B_in["x"],
        "B_w_gate": _B_in["w_gate"],
        "B_w_up": _B_in["w_up"],
        "B_w_down": _B_in["w_down"],
    }

def reference(A_x, A_wqkv, A_wo, B_x, B_w_gate, B_w_up, B_w_down):
    def _A_ref(x, wqkv, wo):
        B, S, D = x.shape
        H = 32; Dh = D // H
        qkv = (lambda x, *d: x.transpose(*d))((x @ wqkv).reshape(B, S, 3, H, Dh), 2, 0, 3, 1, 4)
        q, k, v = qkv[0], qkv[1], qkv[2]
        scale = Dh ** -0.5
        scores = jnp.einsum("bhqd,bhkd->bhqk", q, k) * scale
        p = _softmax(scores, axis=-1)
        o = jnp.einsum("bhqk,bhkd->bhqd", p, v)
        return (lambda x, *d: x.transpose(*d))(o, 0, 2, 1, 3).reshape(B, S, D) @ wo

    def _B_ref(x, w_gate, w_up, w_down):
        g = _silu(x @ w_gate)
        u = x @ w_up
        return (g * u) @ w_down

    x = A_x
    h = x + _A_ref(_layernorm(x, axis=-1), A_wqkv, A_wo)
    h2 = h + _B_ref(_layernorm(h, axis=-1), B_w_gate, B_w_up, B_w_down)
    return h2
```

```python
import math

import jax
import jax.numpy as jnp
import jax.experimental.pallas as pl
import jax.experimental.pallas.tpu as pltpu

_HEADS = 32
_EPS = 1e-5
_RB = 512
_KB = 128
_FB = 256
_HU = 2
_BR = 16
_VPU_BLOCKS = 1
_TRAIL = 2
_RING = 4
_LATE = 2
_SAFE_LO, _SAFE_HI = 2.0 ** -60, 2.0 ** 100
_OP = 4
_P0 = 4
_BF = jnp.bfloat16
_F32 = jnp.float32
_NT = (((1,), (1,)), ((), ()))


def _dot(a, b):
    return jnp.dot(a, b, preferred_element_type=_F32)


def _words(x):
    return pltpu.bitcast(x.astype(_BF), jnp.uint32)


def _halves(w):
    return pltpu.bitcast(w, _BF)


def _add(xs, ys):
    return [x + y for x, y in zip(xs, ys)]


def _layernorm(x):
    xc = x - jnp.mean(x, axis=-1, keepdims=True)
    var = jnp.mean(xc * xc, axis=-1, keepdims=True)
    return xc * jax.lax.rsqrt(var + _EPS)


def _block_kernel(x_hbm, wqkv_hbm, wo_hbm, wg_hbm, wu_hbm, wd_hbm, out_hbm,
                  x_v, wqkv_v, wo_v, wg_v, wu_v, wd_v, out_v,
                  wqvt_v, k_v, qt_v, vt_v, ot_v, qf_v, ks_v, l_v, p_v, h_v, hn_v, a_v,
                  zero_s, x_sem, w_sem, o_sem):
    seq, d = out_hbm.shape
    ff = wg_hbm.shape[1]
    dh = d // _HEADS
    hpg = 128 // dh
    n_rb = seq // _RB
    n_kb = seq // _KB
    n_col = _RB // 128
    n_blk = _KB // _BR
    n_mxu = n_blk - _VPU_BLOCKS
    q_scale = dh ** -0.5 * math.log2(math.e)

    def x_copy(i):
        part = pl.ds(i * n_rb // 2, n_rb // 2)
        return pltpu.make_async_copy(x_hbm.at[part], x_v.at[part], x_sem.at[i])

    def lanes(c):
        return slice(c * 128, (c + 1) * 128)

    out_copies = []
    qkv_copies = [pltpu.make_async_copy(wqkv_hbm.at[:, pl.ds(i * d, d)], wqkv_v.at[i], w_sem.at[i])
                  for i in range(3)]
    ffn_copies = [pltpu.make_async_copy(src, dst, w_sem.at[3 + i]) for i, (src, dst) in enumerate(
        ((wo_hbm, wo_v), (wg_hbm, wg_v), (wu_hbm, wu_v), (wd_hbm, wd_v)))]

    def normalize(c):
        hn_v[c] = _layernorm(x_v[c].astype(_F32)).astype(_BF)

    def project_k(c):
        k = _words(_dot(hn_v[c], wqkv_v[1]))
        for g in range(_HEADS // hpg):
            k_v[g * hpg, c * _RB // 2:(c + 1) * _RB // 2, :] = k[:, lanes(g)]

    def align_keys(c):
        rows = slice(c * _RB // 2, (c + 1) * _RB // 2)
        for h in range(_HEADS):
            if h % hpg:
                k_v[h, rows, :] = pltpu.roll(k_v[h - h % hpg, rows, :], 128 - h % hpg * dh, axis=1)

    def project_q(c):
        qt = jax.lax.dot_general(wqvt_v[0], hn_v[c], _NT, preferred_element_type=_F32)
        qt = (qt * q_scale).astype(_BF)
        qf_v[c] = qt.astype(_F32).reshape(_HEADS, dh, _RB)
        qt_v[c] = _words(qt).reshape(_HEADS, dh // 2, _RB)

    def project_v(c):
        vt = jax.lax.dot_general(wqvt_v[1], hn_v[c], _NT, preferred_element_type=_F32)
        vt_v[:, :, c * _RB:(c + 1) * _RB] = _words(vt).reshape(_HEADS, dh // 2, _RB)

    half = n_rb // 2
    x_copy(0).start()
    qkv_copies[1].start()
    zero_s[0] = 0
    x_copy(0).wait()
    rest = (qkv_copies[0], x_copy(1), qkv_copies[2])
    for cp in rest:
        cp.start()
    qkv_copies[1].wait()
    for c in range(half):
        normalize(c)
        project_k(c)
    for cp in rest:
        cp.wait()
    for cp in ffn_copies:
        cp.start()
    wqvt_v[0] = wqkv_v[0].T
    wqvt_v[1] = wqkv_v[2].T
    for c in range(half):
        project_q(c)
        normalize(half + c)
    for c in range(half, n_rb):
        project_k(c)
        project_q(c)

    n_units = _HU * n_rb
    items = [(kb, b, i) for kb in range(n_kb)
             for b in range(n_mxu, n_blk) for i in range(dh)]
    mxu_blocks = [(u, kb, b) for u in range(n_units) for kb in range(n_kb)
                  for b in range(n_mxu)]
    plan = {blk: [] for blk in mxu_blocks}
    for w in range(n_units * len(items)):
        plan[mxu_blocks[w * len(mxu_blocks) // (n_units * len(items))]].append((w // len(items), w % len(items)))

    def key_rows(kb, b):
        row = ((kb + 1) * _KB - (b + 1) * _BR) // 2
        return slice(row, row + _BR // 2)

    def stage_keys(head, slot, w):
        kb, b, i = items[w]
        k = jnp.broadcast_to(k_v[head, key_rows(kb, b), :][:, i:i + 1], (_BR // 2, 128))
        ks_v[slot][w] = _halves(k).astype(_F32)

    def pv_tile(head, qb, kb, hi, u=None, held=()):
        p = jnp.concatenate([held[u, kb, b] if (u, kb, b) in held else p_v[kb % _RING, n_blk - 1 - b]
                             for b in reversed(range(n_blk))], axis=0).astype(_BF)
        acc = _dot(_halves(vt_v[head, :, kb * _KB:(kb + 1) * _KB]), p)
        if kb > 0:
            acc = ot_v[qb, head] + acc
        ot_v[qb, head] = acc
        if kb == n_kb - 1:
            for c in range(n_col):
                mag = jnp.abs(acc[:, lanes(c)])
                hi = jnp.maximum(hi, jnp.maximum(mag[:8], mag[8:]))
        return hi

    def attend_unshifted(step, state):
        lo, hi = state
        keep = jnp.full((8, 128), zero_s[0], jnp.int32) == 0
        seen, late, held = [], [], {}

        def paced(x, c):
            return jnp.where(keep, x, seen[-1][c % n_col])

        def weights(where, s):
            e = [jnp.exp2(x) for x in s]
            u, kb, b = where
            if b < n_blk // 2 or (u == n_units - 1 and kb >= n_kb - _TRAIL):
                p_v[kb % _RING, n_blk - 1 - b] = jnp.concatenate(e, axis=1)
            else:
                held[where] = jnp.concatenate(e, axis=1)
            return [x[:8] + x[8:] for x in e]

        for u in range(n_units):
            head, qb = step * _HU + u // n_rb, u % n_rb
            l = None
            for kb in range(n_kb):
                k = jnp.concatenate([k_v[head, key_rows(kb, b), :] for b in range(n_mxu)], axis=0)
                s = _dot(_halves(k)[:, :dh], _halves(qt_v[qb, head]))
                for b in range(n_mxu):
                    t = weights((u, kb, b), [s[b * _BR:(b + 1) * _BR, lanes(c)] for c in range(n_col)])
                    l = t if l is None else _add(l, t)
                    if late and late[0][0] == u and late[0][1] <= len(seen):
                        l = _add(l, late.pop(0)[2])
                    seen.append(l)
                    for vu, w in plan[u, kb, b]:
                        vk, vb, i = items[w]
                        kk = ks_v[vu // n_rb % 2][w]
                        kk = jnp.concatenate([paced(kk[:8], 2 * i), paced(kk[8:], 2 * i + 1)], axis=0)
                        t = [kk * qf_v[vu % n_rb, step * _HU + vu // n_rb, i:i + 1, lanes(c)]
                             for c in range(n_col)]
                        sv = t if i == 0 else _add(sv, t)
                        if i == dh - 1:
                            late.append((vu, len(seen) + _LATE, weights((vu, vk, vb), sv)))
                for w in range(len(items)):
                    if w * n_rb * n_kb // len(items) == qb * n_kb + kb:
                        stage_keys((head + 1) % _HEADS, (u // n_rb + 1) % 2, w)
                if kb >= _TRAIL:
                    hi = pv_tile(head, qb, kb - _TRAIL, hi, u, held)
                else:
                    hi = pv_tile((head + _HEADS - (qb == 0)) % _HEADS, (qb - 1) % n_rb,
                                 n_kb + kb - _TRAIL, hi, u - 1, held)
            while late and late[0][0] == u:
                l = _add(l, late.pop(0)[2])
            l_v[qb, head] = jnp.concatenate(l, axis=1)
            for x in l:
                lo, hi = jnp.minimum(lo, x), jnp.maximum(hi, x)
        return lo, hi

    def attend_exact(u, carry):
        head, qb = u // n_rb, u % n_rb
        q = _halves(qt_v[qb, head])

        def scores(kb):
            k = _halves(k_v[head, pl.ds(pl.multiple_of(kb * (_KB // 2), _KB // 2), _KB // 2), :])
            return _dot(k[:, :dh], q)

        m = jax.lax.fori_loop(
            0, n_kb, lambda kb, m: jnp.maximum(m, jnp.max(scores(kb), axis=0, keepdims=True)),
            jnp.full((1, _RB), -jnp.inf, _F32))
        l, acc = jnp.zeros((8, _RB), _F32), jnp.zeros((dh, _RB), _F32)
        for kb in range(n_kb):
            p = jnp.exp2(scores(kb) - m)
            l = l + jnp.sum(p.reshape(-1, 8, _RB), axis=0)
            acc = acc + _dot(_halves(vt_v[head, :, kb * _KB:(kb + 1) * _KB]), p.astype(_BF))
        l_v[qb, head] = l
        ot_v[qb, head] = acc
        return carry

    for w in range(len(items)):
        stage_keys(0, 0, w)
    for c in range(n_rb):
        align_keys(c)
        project_v(c)
    ot_v[n_rb - 1, _HEADS - 1] = jnp.zeros((dh, _RB), _F32)
    for kb in range(n_kb - _TRAIL, n_kb):
        p_v[kb % _RING] = jnp.zeros(p_v.shape[1:], p_v.dtype)
    ones = jnp.ones((8, 128), _F32)
    lo, hi = jax.lax.fori_loop(0, _HEADS // _HU, attend_unshifted, (ones, ones))
    for kb in range(n_kb - _TRAIL, n_kb):
        hi = pv_tile(_HEADS - 1, n_rb - 1, kb, hi)
    safe = jnp.logical_and(lo >= _SAFE_LO, hi <= _SAFE_HI)
    n_unsafe = jnp.sum(jnp.where(safe, 0.0, 1.0))

    for cp in ffn_copies:
        cp.wait()

    def project(c):
        o = ot_v[c] * (1.0 / jnp.sum(l_v[c], axis=1, keepdims=True))
        h = x_v[c].astype(_F32) + _dot(o.reshape(d, _RB).astype(_BF).T, wo_v[...])
        h_v[c] = h
        hn_v[c] = _layernorm(h).astype(_BF)

    def gate(c, f):
        fs = slice(f * _FB, (f + 1) * _FB)
        g = _dot(hn_v[c], wg_v[:, fs])
        u = _dot(hn_v[c], wu_v[:, fs])
        a_v[:, fs] = (g * jax.nn.sigmoid(g) * u).astype(_BF)

    for c in range(_P0):
        project(c)
    for c in range(n_rb):
        if c and c + _P0 - 1 < n_rb:
            project(c + _P0 - 1)
        for f in range(ff // _FB):
            gate(c, f)
            if f == 1 and c:
                out_copies[-1].start()
        parts = _OP if c + 1 == n_rb else 1
        for i in range(parts):
            rows = slice(i * _RB // parts, (i + 1) * _RB // parts)
            out_v[c, rows] = (h_v[c, rows] + _dot(a_v[rows, :], wd_v[...])).astype(out_v.dtype)
            out_copies.append(pltpu.make_async_copy(
                out_v.at[c, rows], out_hbm.at[pl.ds(c * _RB + rows.start, _RB // parts)],
                o_sem.at[len(out_copies)]))
            if c + 1 == n_rb:
                out_copies[-1].start()
    for cp in out_copies:
        cp.wait()

    @pl.when(n_unsafe > 0.0)
    def _():
        jax.lax.fori_loop(0, _HEADS * n_rb, attend_exact, 0)

        def redo(c, carry):
            project(c)
            for f in range(ff // _FB):
                gate(c, f)
            out_v[c] = (h_v[c] + _dot(a_v[...], wd_v[...])).astype(out_v.dtype)
            cp = pltpu.make_async_copy(
                out_v.at[c], out_hbm.at[pl.ds(pl.multiple_of(c * _RB, _RB), _RB)], o_sem.at[0])
            cp.start()
            cp.wait()
            return carry

        jax.lax.fori_loop(0, n_rb, redo, 0)


@jax.jit
def pallas_sequential_preLN__softmax_full_mha__swiglu_ffn__prompt_kernel(
    A_x: jax.Array,
    A_wqkv: jax.Array,
    A_wo: jax.Array,
    B_x: jax.Array,
    B_w_gate: jax.Array,
    B_w_up: jax.Array,
    B_w_down: jax.Array,
):
    del B_x
    batch, seq, d = A_x.shape
    assert batch == 1
    ff = B_w_gate.shape[1]
    dh = d // _HEADS
    n_rb = seq // _RB
    vmem = pltpu.VMEM
    out = pl.pallas_call(
        _block_kernel,
        out_shape=jax.ShapeDtypeStruct((seq, d), A_x.dtype),
        in_specs=[pl.BlockSpec(memory_space=pl.ANY)] * 6,
        out_specs=pl.BlockSpec(memory_space=pl.ANY),
        scratch_shapes=[
            vmem((n_rb, _RB, d), A_x.dtype),
            vmem((3, d, d), A_wqkv.dtype),
            vmem(A_wo.shape, A_wo.dtype),
            vmem(B_w_gate.shape, B_w_gate.dtype),
            vmem(B_w_up.shape, B_w_up.dtype),
            vmem(B_w_down.shape, B_w_down.dtype),
            vmem((n_rb, _RB, d), A_x.dtype),
            vmem((2, d, d), _BF),
            vmem((_HEADS, seq // 2, 128), jnp.uint32),
            vmem((n_rb, _HEADS, dh // 2, _RB), jnp.uint32),
            vmem((_HEADS, dh // 2, seq), jnp.uint32),
            vmem((n_rb, _HEADS, dh, _RB), _F32),
            vmem((n_rb, _HEADS, dh, _RB), _F32),
            [vmem((seq // _KB * _VPU_BLOCKS * dh, _BR, 128), _F32)] * 2,
            vmem((n_rb, _HEADS, 8, _RB), _F32),
            vmem((_RING, _KB // _BR, _BR, _RB), _F32),
            vmem((n_rb, _RB, d), _F32),
            vmem((n_rb, _RB, d), _BF),
            vmem((_RB, ff), _BF),
            pltpu.SMEM((1,), jnp.int32),
            pltpu.SemaphoreType.DMA((2,)),
            pltpu.SemaphoreType.DMA((7,)),
            pltpu.SemaphoreType.DMA((n_rb - 1 + _OP,)),
        ],
        compiler_params=pltpu.CompilerParams(vmem_limit_bytes=100 * 2**20),
        name="tblock",
    )(A_x.reshape(n_rb, _RB, d), A_wqkv, A_wo, B_w_gate, B_w_up, B_w_down)
    return out.reshape(batch, seq, d)
```
